```python
import os as _os
_os.environ.setdefault("JAX_PLATFORMS", "cpu")
import jax
import jax.numpy as jnp

def _softmax(x, axis=-1):
    return jax.nn.softmax(x, axis=axis)
def _gelu(x):
    return jax.nn.gelu(x, approximate=True)
def _silu(x):
    return jax.nn.silu(x)
def _sigmoid(x):
    return jax.nn.sigmoid(x)
def _layernorm(x, axis=-1, eps=1e-5):
    m = jnp.mean(x, axis=axis, keepdims=True)
    v = jnp.var(x, axis=axis, keepdims=True)
    return (x - m) / jnp.sqrt(v + eps)
def _scatter_add(tgt, idx, src, axis=0):
    return tgt.at[idx].add(src)
def _segment_sum(src, seg, n):
    return jax.ops.segment_sum(src, seg, n)
class _Rng:
    def __init__(self, key):
        self._k = key
    def _next(self):
        self._k, sub = jax.random.split(self._k)
        return sub
    def normal(self, shape):
        return jax.random.normal(self._next(), shape, dtype=jnp.bfloat16)
    def randint(self, lo, hi, shape):
        return jax.random.randint(self._next(), shape, lo, hi, dtype=jnp.int32)
    def uniform(self, shape, lo=0.0, hi=1.0):
        return jax.random.uniform(self._next(), shape, jnp.bfloat16, lo, hi)
    def permutation(self, n):
        return jax.random.permutation(self._next(), n)


kernel_name = 'standalone__fft_conv__vision'

def setup_inputs():
    _rng = _Rng(jax.random.key(int.from_bytes(__import__("os").urandom(4), "little")))
    _w = (lambda a: (lambda t: t.astype(jnp.bfloat16) if jnp.issubdtype(t.dtype, jnp.floating) else t)(jnp.asarray(a)))
    H = W = 224
    C = 96
    K = 3
    return {
        "x": _w((lambda *s: _rng.normal(s) * 0.05)(1, H, W, C)),
        "w": _w((lambda *s: _rng.normal(s) * 0.05)(K, K, C, C)),
    }

def reference(x, w):
    B, H, W, C = x.shape
    K = w.shape[0]
    wp = jnp.pad(w, ((0, H - K), (0, W - K), (0, 0), (0, 0)))
    Xf = (lambda x, axes=(-2,-1): jnp.fft.rfft2(x.astype(jnp.float32), axes=axes))(x, axes=(1, 2))
    Wf = (lambda x, axes=(-2,-1): jnp.fft.rfft2(x.astype(jnp.float32), axes=axes))(wp, axes=(0, 1))
    Yf = jnp.einsum('bhwi,hwio->bhwo', Xf, Wf)
    y = (lambda x, s, axes=(-2,-1): jnp.fft.irfft2(x, s=s, axes=axes).astype(jnp.bfloat16))(Yf, (H, W), axes=(1, 2))
    return y
```

```python
import functools
import numpy as np
import jax, jax.numpy as jnp
from jax import lax
from jax.experimental import pallas as pl
from jax.experimental.pallas import tpu as pltpu

H, C, W = 224, 96, 224
NG = H // 4
F32, BF16, U32 = jnp.float32, jnp.bfloat16, jnp.uint32

def make(a=2/3, b=None, rd=(24, 32, 40, 56, 64, 8), wr=(128, 64, 24, 8), G=1, D=4, nodma=False, nord=False, nowr=False, flags=None, ofirst=False, fine=True):
    b = 1.0 / a if b is None else b
    nord = nord or nodma; nowr = nowr or nodma
    pts = [0.0, a, -a, b, -b]
    GH = np.zeros((6, 3))
    for j, p in enumerate(pts):
        f = np.prod([p - q for k, q in enumerate(pts) if k != j])
        GH[j] = [p ** k / f for k in range(3)]
    GH[5, 2] = 1.0
    rd_edges = np.cumsum((0,) + tuple(rd)); wr_edges = np.cumsum((0,) + tuple(wr))
    assert rd_edges[-1] == H and wr_edges[-1] == H
    NP = NG // G
    VR = 6 * G * C
    mul = lambda v, c: v if abs(c - 1.0) < 1e-12 else v * c

    def kernel(x_hbm, w_hbm, o_hbm, xb, yb, wb, ub, rr, va, vb, ma, mb, cb, sem_w, sem_r, sem_o):
        va = va.bitcast(BF16); vb = vb.bitcast(BF16)
        def rd_copy(i):
            s, n = int(rd_edges[i]), int(rd[i])
            return pltpu.make_async_copy(x_hbm.at[pl.ds(s, n)], xb.at[pl.ds(s, n)], sem_r.at[i])
        def wr_copy(i):
            s, n = int(wr_edges[i]), int(wr[i])
            return pltpu.make_async_copy(yb.at[pl.ds(s, n)], o_hbm.at[pl.ds(s, n)], sem_o.at[i])
        w_copy = pltpu.make_async_copy(w_hbm, wb, sem_w.at[0])
        halo = lambda: pltpu.make_async_copy(x_hbm.at[pl.ds(H - 2, 2)], xb.at[pl.ds(H, 2)], sem_w.at[1])
        w_copy.start()
        if not nord:
            halo().start()
            for i in range(len(rd)):
                rd_copy(i).start()
        w_copy.wait()

        g = [[wb[2 - k, 2 - l].astype(F32).T for l in range(3)] for k in range(3)]
        for wc in range(4):
            col = []
            for k in range(3):
                if wc == 0: col.append(g[k][0])
                elif wc == 3: col.append(g[k][2])
                elif wc == 1: col.append((g[k][0] + g[k][2] + g[k][1]) * 0.5)
                else: col.append((g[k][0] + g[k][2] - g[k][1]) * 0.5)
            for hc in range(6):
                u = None
                for k in range(3):
                    c = float(GH[hc, k])
                    if c == 0.0: continue
                    t = mul(col[k], c)
                    u = t if u is None else u + t
                ub[hc * 4 + wc] = pltpu.bitcast(u.astype(BF16), U32)

        def masks(n):
            lane = lax.broadcasted_iota(jnp.int32, (n, 128), 1)
            even = (lane & 1) == 0
            odd = (lane & 1) == 1
            mid = (lane >= 96) & (lane < 126)
            top = lane >= 126
            return mid | (even ^ top), mid | (odd ^ top), even ^ top, even
        m_f, m_g, _, _ = masks(8)
        _, _, m_o, m_e = masks(16)

        def wrap(row, s):
            r = pltpu.bitcast(xb[row, pl.ds(16 * s, 16), pl.ds(128, 96)], U32)
            return jnp.concatenate([r, r[:, 64:96]], axis=1)

        def w_in(row, s, r):
            l = pltpu.bitcast(xb[row, pl.ds(16 * s, 16), pl.ds(0, 128)], U32)
            f = jnp.where(m_f, l, r)
            gg = jnp.where(m_g, l, r)
            up = lambda v: pltpu.bitcast(v, BF16).astype(F32)
            d0 = up(pltpu.roll(f, 2, 1)); d1 = up(pltpu.roll(gg, 1, 1)); d2 = up(f); d3 = up(pltpu.roll(gg, 127, 1))
            return [d0 - d2, d1 + d2, d2 - d1, d1 - d3]

        def h_in(d):
            if a == 1.0:
                p = d[4] - d[2] * (b * b); q = d[3] - d[1] * (b * b)
                r = d[4] - d[2]; u = (d[3] - d[1]) * b
                return [(d[0] - d[2]) * (b * b) + r, p + q, p - q, r + u, r - u, (d[5] - d[3]) - u * b]
            al = d[2] * (a * a); be = d[2] * (b * b)
            p = d[4] - be; r = d[4] - al
            t0 = d[0] + (p - al)
            q = d[3] * a - d[1] * b
            u = d[3] * b - d[1] * a
            t5 = (d[1] + d[5]) - d[3] * (a * a + b * b)
            return [t0, p + q, p - q, r + u, r - u, t5]

        def h_stage(rows, k, v, s):
            for wc in range(4):
                d = [cb[0, wc, pl.ds(16 * s, 16), :], cb[1, wc, pl.ds(16 * s, 16), :]] + [rows[r][wc] for r in range(4)]
                cb[0, wc, pl.ds(16 * s, 16), :] = d[4]
                cb[1, wc, pl.ds(16 * s, 16), :] = d[5]
                for hc, t in enumerate(h_in(d)):
                    v[pl.ds((k * 6 + hc) * C + 16 * s, 16), pl.ds(128 * wc, 128)] = t.astype(BF16)

        def stage_mm(v, m, k, hc):
            p = [jnp.dot(pltpu.bitcast(ub[hc * 4 + wc], BF16), v[pl.ds((k * 6 + hc) * C, C), pl.ds(128 * wc, 128)],
                         preferred_element_type=F32) for wc in range(4)]
            m[k, hc] = jnp.concatenate([p[0] + p[1] + p[2], p[1] - p[2] - p[3]], axis=1)

        def h_out(m, k, s):
            t = [m[k, hc, pl.ds(16 * s, 16), :] for hc in range(6)]
            s1 = t[1] + t[2]; d1 = t[1] - t[2]; s2 = t[3] + t[4]; d2 = t[3] - t[4]
            return [s1 + s2 + t[0], mul(d1, a) + d2 * b, mul(s1, a * a) + s2 * (b * b), mul(d1, a ** 3) + d2 * (b ** 3) + t[5]]

        def put(row, s, y):
            y0 = y[:, :128]; z = pltpu.roll(y[:, 128:], 1, 1)
            y = jnp.concatenate([jnp.where(m_o, y0, z), jnp.where(m_e, z, y0)[:, :96]], axis=1)
            yb[row, pl.ds(16 * s, 16), :] = y.astype(BF16)

        NU = 24 * G
        def unit(t, j):
            if j >= NU: t, j = jnp.minimum(t + 1, NP - 1) if not isinstance(t, int) else t + 1, j - NU
            return 4 * G * t + 4 * (j // 24) + j % 4, (j // 4) % 6

        def phase(t, par, in_=True, mm_=True, out_=True):
            m0, m1 = (ma, mb) if par == 0 else (mb, ma)
            v0, v1 = (va, vb) if par == 0 else (vb, va)
            q = [rr[i] for i in range(D)] if in_ else None
            for u in range(6 * G):
                k, s = u // 6, u % 6
                if mm_: stage_mm(v1, m1, k, s)
                ys = h_out(m0, k, s) if out_ else None
                rows = []
                o = lambda r: put(4 * (G * (t - 2) + k) + r, s, ys[r])
                if out_ and not fine and ofirst:
                    for r in range(4): o(r)
                for r in range(4):
                    if out_ and fine and ofirst: o(r)
                    if in_:
                        q.append(wrap(*unit(t, 4 * u + r + D)))
                        rows.append(w_in(*unit(t, 4 * u + r), q.pop(0)))
                    if out_ and fine and not ofirst: o(r)
                if out_ and not fine and not ofirst:
                    for r in range(4): o(r)
                if in_: h_stage(rows, k, v0, s)
            if in_:
                for i in range(D): rr[i] = q[i]

        if not nord:
            halo().wait()
            rd_copy(0).wait()
        hw = [[wrap(H + r, s) for r in range(2)] for s in range(6)]
        for i in range(D): rr[i] = wrap(*unit(0, i))
        for s in range(6):
            for r in range(2):
                for wc, t in enumerate(w_in(H + r, s, hw[s][r])):
                    cb[r, wc, pl.ds(16 * s, 16), :] = t
        phase(0, 0, mm_=False, out_=False)
        phase(1, 1, out_=False)
        wr_at = [-(-int(wr_edges[i + 1]) // (4 * G)) + 2 for i in range(len(wr))]
        def body(t, _):
            if not nord:
                for i in range(1, len(rd)):
                    first = max(int(rd_edges[i]) // (4 * G) - 1, 2)
                    pl.when(t == first)(lambda i=i: rd_copy(i).wait())
            if not nowr:
                for i in range(len(wr)):
                    if wr_at[i] < NP:
                        pl.when(t == wr_at[i])(lambda i=i: wr_copy(i).start())
            pl.when(t % 2 == 0)(lambda: phase(t, 0))
            pl.when(t % 2 == 1)(lambda: phase(t, 1))
        lax.fori_loop(2, NP, body, None)
        def start_at(t):
            if not nowr:
                for i in range(len(wr)):
                    if wr_at[i] == t: wr_copy(i).start()
        start_at(NP)
        phase(NP, NP % 2, in_=False)
        start_at(NP + 1)
        phase(NP + 1, (NP + 1) % 2, in_=False, mm_=False)
        start_at(NP + 2)
        if not nowr:
            assert max(wr_at) <= NP + 2 and min(wr_at) >= 2
            for i in range(len(wr)):
                wr_copy(i).wait()

    def f(x, w):
        xt = jnp.transpose(x, (0, 1, 3, 2)).reshape(H, C, W)
        y = pl.pallas_call(
            kernel,
            in_specs=[pl.BlockSpec(memory_space=pl.ANY), pl.BlockSpec(memory_space=pl.ANY)],
            out_specs=pl.BlockSpec(memory_space=pl.ANY),
            out_shape=jax.ShapeDtypeStruct((H, C, W), BF16),
            scratch_shapes=[
                pltpu.VMEM((H + 2, C, W), BF16), pltpu.VMEM((H, C, W), BF16), pltpu.VMEM((3, 3, C, C), BF16),
                pltpu.VMEM((24, C // 2, C), U32),
                pltpu.VMEM((D, 8, 128), U32),
                pltpu.VMEM((VR // 2, 512), U32), pltpu.VMEM((VR // 2, 512), U32),
                pltpu.VMEM((G, 6, C, 256), F32), pltpu.VMEM((G, 6, C, 256), F32),
                pltpu.VMEM((2, 4, C, 128), F32),
                pltpu.SemaphoreType.DMA((2,)), pltpu.SemaphoreType.DMA((len(rd),)), pltpu.SemaphoreType.DMA((len(wr),)),
            ],
            compiler_params=pltpu.CompilerParams(vmem_limit_bytes=64 * 2 ** 20, flags=flags),
        )(xt, w)
        return jnp.transpose(y.reshape(1, H, C, W), (0, 1, 3, 2))
    return f


_impl = make(D=4, G=2, wr=(80, 56, 32, 24, 16, 8, 8))

@jax.jit
def pallas_standalone__fft_conv__vision_kernel(x, w):
    return _impl(x, w)
```

```python
import functools

import jax
import jax.experimental.pallas as pl
import jax.experimental.pallas.tpu as pltpu
import jax.numpy as jnp
import numpy as np
from jax import lax

H, W, C, K = 224, 224, 96, 3
F32, BF16, U32 = jnp.float32, jnp.bfloat16, jnp.uint32

BANDS = 4
BAND_ROWS = H // BANDS
STEPS = BAND_ROWS // 4
SLABS = C // 16
STEP = 4 * C

A = (5.0**0.5 - 1.0) / 2.0
B = A + 1.0


def _filter_coefficients(p):
    norm = np.prod([p - q for q in (0.0, A, -A, B, -B) if q != p])
    return [float(p ** (k + 1) / norm) for k in range(K)]


DMA_ORDER = (0, 2, 1, 3)
READ_ITERS = 6
READ_ROWS = 7
EARLY_ROWS = BAND_ROWS - 2 - READ_ITERS * READ_ROWS
PIECE = 64
OLD_PIECES = 4
assert EARLY_ROWS == 12
assert OLD_PIECES * PIECE * (STEPS - 2 - READ_ITERS) == STEP * (READ_ITERS - 2)

READY_ROUNDS = 2
SLOT_AFTER = (0, 2, 3, 5)
IN_BAND_ORDER = (1, 2, 3, 0)
IN_DELAY, OUT_DELAY, READY_DELAY = 6, 4, 8


def _h_forward(d):
    s = d[2] * (A * A)
    p = d[4] - d[2] * (B * B)
    r = d[4] - s
    e = (d[3] - d[1]) * A
    q = e - d[1]
    u = e + d[3]
    return [d[0] + (p - s), p + q, p - q, r + u, r - u, (d[1] + d[5]) - d[3] * 3.0]


def _h_inverse(m):
    s1, d1 = m[1] + m[2], m[1] - m[2]
    s2, d2 = m[3] + m[4], m[3] - m[4]
    e = (s1 + s2) * A
    return [e + s1 + m[0], d1 + d2, e + s2, d1 * (A * A) + d2 * (B * B) + m[5]]


def _w_forward(t):
    d1, d2 = t[:, :128], t[:, 128:]
    return [pltpu.roll(d2, 2, 1) - d2, d1 + d2, d2 - d1, d1 - pltpu.roll(d1, 126, 1)]


def _w_inverse(p):
    return jnp.concatenate([p[0] + p[1] + p[2], p[1] - p[2] - p[3]], axis=1)


def _ds(start, size):
    return pl.ds(start if isinstance(start, int) else pl.multiple_of(start, 16), size)


def _slab(s):
    return pl.ds(16 * s, 16)


def _prepare_filter(w_buf, taps, u_buf):
    for a in range(K):
        for b in range(K):
            taps[a, b] = w_buf[K - 1 - a, K - 1 - b].astype(F32).T

    def body(s, _):
        rows = []
        for a in range(K):
            g0, g1, g2 = (taps[a, b, _ds(16 * s, 16), :] for b in range(K))
            even, odd = (g0 + g2) * 0.5, g1 * 0.5
            rows.append([g0, even + odd, even - odd, g2])
        for wc in range(4):
            g0, g1, g2 = (rows[a][wc] for a in range(K))
            parts = [g0]
            for p in (A, B):
                c0, c1, c2 = _filter_coefficients(p)
                even, odd = g0 * c0 + g2 * c2, g1 * c1
                parts += [even + odd, even - odd]
            parts.append(g2)
            for hc, u in enumerate(parts):
                u_buf[_ds(hc * C + 16 * s, 16), pl.ds(128 * wc, C)] = u.astype(BF16)

    lax.fori_loop(0, SLABS, body, None)


def _compute(
    x_hbm, w_hbm, y_hbm,
    x_buf, y_buf, w_buf, taps, u_buf, t_even, t_odd, v_even, v_odd, m_even, m_odd, carry,
    write_sem, early_sems, read_sems,
):
    u_buf, v_even, v_odd = (r.bitcast(BF16) for r in (u_buf, v_even, v_odd))
    all_bands = slice(None)

    def read(band, start, size, sem):
        where = (band, pl.ds(start, size))
        return pltpu.make_async_copy(x_hbm.at[where], x_buf.at[where], sem)

    def write(band, start, size):
        src, dst = y_buf.at[band, pl.ds(STEP + start, size)], y_hbm.at[band, pl.ds(start, size)]
        pltpu.make_async_copy(src, dst, write_sem).start()

    def first_rows(k):
        sem = early_sems.at[k]
        return read((k + BANDS - 1) % BANDS, (BAND_ROWS - 2) * C, 2 * C, sem), read(k, 0, STEP, sem)

    w_copy = pltpu.make_async_copy(w_hbm, w_buf, early_sems.at[BANDS + 1])
    w_copy.start()
    for k in range(BANDS):
        for copy in first_rows(k):
            copy.start()
    for k in range(BANDS):
        read(k, STEP, STEP, early_sems.at[BANDS]).start()
    for k in range(BANDS):
        read(k, 2 * STEP, STEP, read_sems.at[0]).start()

    def clear(k, _):
        m_odd[k] = jnp.zeros(m_odd.shape[1:], F32)

    lax.fori_loop(0, BANDS, clear, None)
    w_copy.wait()
    _prepare_filter(w_buf, taps, u_buf)

    def lane_masks(rows):
        lane = lax.broadcasted_iota(jnp.int32, (rows, 128), 1)
        return (lane & 1) == 0, (lane & 1) == 1, (lane >= 96) & (lane < 126), lane >= 126

    even, odd, middle, top = lane_masks(8)
    own_from_left, other_from_left = middle | (even ^ top), middle | (odd ^ top)
    even, _, _, top = lane_masks(16)
    left_is_first, right_is_second = even ^ top, even

    def load_right(ref, band, line):
        r = pltpu.bitcast(ref[band, pl.ds(line, 16), pl.ds(128, W - 128)], U32)
        return jnp.concatenate([r, r[:, 64:]], axis=1)

    def load_pixels(ref, band, line, right):
        left = pltpu.bitcast(ref[band, pl.ds(line, 16), pl.ds(0, 128)], U32)
        before = pltpu.roll(jnp.where(other_from_left, left, right), 1, 1)
        own = jnp.where(own_from_left, left, right)
        return jnp.concatenate([pltpu.bitcast(v, BF16).astype(F32) for v in (before, own)], axis=1)

    def store_pixels(ref, band, line, y):
        first, second = y[:, :128], pltpu.roll(y[:, 128:], 1, 1)
        left = jnp.where(left_is_first, first, second)
        right = jnp.where(right_is_second, second, first)[:, : W - 128]
        ref[band, pl.ds(line, 16), :] = jnp.concatenate([left, right], axis=1).astype(BF16)

    def keep(t_buf, v_buf, band, s, parts):
        for hc, t in enumerate(parts):
            if band == 0 and hc < READY_ROUNDS:
                for wc, v in enumerate(_w_forward(t)):
                    v_buf[pl.ds(hc * C + 16 * s, 16), pl.ds(128 * wc, 128)] = v.astype(BF16)
            else:
                t_buf[band, hc, _slab(s), :] = t

    def iteration(i, parity, reading=False):
        closing = isinstance(i, int)
        last = closing and i == STEPS
        t_new, t_old = (t_even, t_odd)[:: 1 - 2 * parity]
        v_new, v_old = (v_even, v_odd)[:: 1 - 2 * parity]
        m_old, m_new = (m_even, m_odd)[:: 1 - 2 * parity]
        units = 4 * SLABS * BANDS

        agenda = {}

        def plan(slot, fn, *args):
            agenda.setdefault(slot, []).append(functools.partial(fn, *args))

        def plan_forward():
            x_step = x_buf.at[:, _ds(STEP * i, STEP)]
            rights, rows = [], []

            def unit(j, band, s, r):
                if r == 0:
                    rows[:] = [carry[band, 0, _slab(s), :], carry[band, 1, _slab(s), :]]
                rows.append(load_pixels(x_step, band, r * C + 16 * s, rights.pop(0)))
                if r == 3:
                    carry[band, 0, _slab(s), :] = rows[4]
                    carry[band, 1, _slab(s), :] = rows[5]
                    args = (t_new, v_new, band, s, _h_forward(rows))
                    if band == 0:
                        plan(j + IN_DELAY + READY_DELAY, keep, *args)
                    else:
                        keep(*args)

            for j in range(units):
                band, s, r = IN_BAND_ORDER[j // (4 * SLABS)], j // 4 % SLABS, j % 4
                plan(j, lambda *a: rights.append(load_right(*a)), x_step, band, r * C + 16 * s)
                plan(j + IN_DELAY, unit, j, band, s, r)

        def plan_inverse(m_buf, step, slot, band_major):
            y_step = y_buf.at[:, _ds(STEP * (step + 1), STEP)]
            rows = []

            def unit(j):
                r = j % 4
                band, s = (j // (4 * SLABS), j // 4 % SLABS) if band_major else (j // 4 % BANDS, j // (4 * BANDS))
                if r == 0:
                    rows[:] = _h_inverse([m_buf[band, hc, _slab(s), :] for hc in range(6)])
                store_pixels(y_step, band, r * C + 16 * s, rows[r])
                if closing and (j + 1) % (units // 2) == 0:
                    for line in range(STEP * step, STEP * (step + 1), C):
                        if band_major:
                            write(band - 1, line, C)
                            write(band, line, C)
                        else:
                            for k in DMA_ORDER:
                                write(k, line + 16 * (s + 1) - C // 2, C // 2)

            for j in range(units):
                plan(slot(j), unit, j)

        if last:
            plan_inverse(m_old, i - 2, lambda j: j // 2, False)
            plan_inverse(m_new, i - 1, lambda j: max(48 + j // 2, 24 * (j // 24) + 36 + j % 24 // 2), True)
        else:
            plan_forward()
            plan_inverse(m_old, i - 2, lambda j: j + OUT_DELAY, not closing)

        def start_piece(src, dst, n, size, sem, priority):
            where = (DMA_ORDER[n % BANDS], pl.ds(n // BANDS * size, size))
            pltpu.make_async_copy(src.at[where], dst.at[where], sem).start(priority=priority)

        if reading:
            span = _ds((EARLY_ROWS + (i - 1) * READ_ROWS) * C, READ_ROWS * C)
            count = BANDS * READ_ROWS
            for n in range(count):
                args = (x_hbm.at[:, span], x_buf.at[:, span], n, C, read_sems.at[i], n % 2)
                plan(n * 100 // count, start_piece, *args)
        elif not closing:
            spans = [((i - READ_ITERS - 1) * OLD_PIECES * PIECE, OLD_PIECES * PIECE), ((i - 3) * STEP, STEP)]
            pieces = sorted(
                ((n + 0.5) * PIECE / size, which, n)
                for which, (_, size) in enumerate(spans)
                for n in range(size // PIECE)
            )
            count = BANDS * len(pieces)
            for n in range(count):
                _, which, piece = pieces[n // BANDS]
                start, size = spans[which]
                src, dst = y_buf.at[:, _ds(STEP + start, size)], y_hbm.at[:, _ds(start, size)]
                plan(12 + n * 68 // count, start_piece, src, dst, BANDS * piece + n % BANDS, PIECE, write_sem, 0)
        elif not last:
            count = BANDS * STEP // PIECE
            for n in range(count):
                plan(n * 32 // count, write, DMA_ORDER[n % BANDS], (i - 3) * STEP + n // BANDS * PIECE, PIECE)

        slot = 0

        def emit():
            nonlocal slot
            for fn in agenda.pop(slot, []):
                fn()
            slot += 1

        for band in range(BANDS):
            for hc in range(6):
                if band == 0 and hc < READY_ROUNDS:
                    v = [v_old[pl.ds(hc * C, C), pl.ds(128 * wc, 128)] for wc in range(4)]
                    for _ in SLOT_AFTER:
                        emit()
                else:
                    slabs = []
                    for n in range(SLABS):
                        slabs.insert(0, _w_forward(t_old[band, hc, _slab(SLABS - 1 - n), :]))
                        if n in SLOT_AFTER:
                            emit()
                    v = [jnp.concatenate(part, axis=0).astype(BF16) for part in zip(*slabs)]
                m_new[band, hc] = _w_inverse([
                    jnp.dot(u_buf[pl.ds(hc * C, C), pl.ds(128 * wc, C)], v[wc], preferred_element_type=F32)
                    for wc in range(4)
                ])
        while agenda:
            emit()

    def first_step(k, _):
        for copy in first_rows(k):
            copy.wait()
        above = (k + BANDS - 1) % BANDS
        lines = [(above, (BAND_ROWS - 2 + r) * C) for r in range(2)] + [(k, r * C) for r in range(4)]
        rights = [[load_right(x_buf, band, line + 16 * s) for band, line in lines] for s in range(SLABS)]
        for s in range(SLABS):
            rows = [load_pixels(x_buf, band, line + 16 * s, r) for (band, line), r in zip(lines, rights[s])]
            carry[k, 0, _slab(s), :] = rows[4]
            carry[k, 1, _slab(s), :] = rows[5]
            for hc, t in enumerate(_h_forward(rows)):
                t_even[k, hc, _slab(s), :] = t

    lax.fori_loop(0, BANDS, first_step, None)
    for s in range(SLABS):
        keep(t_even, v_even, 0, s, [t_even[0, hc, _slab(s), :] for hc in range(READY_ROUNDS)])
    read(all_bands, STEP, STEP, early_sems.at[BANDS]).wait()

    edges = [8] + [EARLY_ROWS + b * READ_ROWS for b in range(READ_ITERS + 1)]
    assert all(b < edges[b] // 4 < STEPS - 1 for b in range(READ_ITERS + 1))

    def run(begin, end, reading):
        def body(i, _):
            for b, (lo, hi) in enumerate(zip(edges, edges[1:])):
                if begin <= lo // 4 < end:
                    pl.when(i == lo // 4)(read(all_bands, lo * C, (hi - lo) * C, read_sems.at[b]).wait)
            lax.cond((i & 1) == 0, lambda: iteration(i, 0, reading), lambda: iteration(i, 1, reading))

        lax.fori_loop(begin, end, body, None)

    run(1, READ_ITERS + 1, True)
    run(READ_ITERS + 1, STEPS - 1, False)
    closing = [functools.partial(iteration, i, i % 2) for i in (STEPS - 1, STEPS)]
    lax.fori_loop(0, 2, lambda n, _: lax.switch(n, closing), None)


def _kernel(x_hbm, w_hbm, y_hbm, x_buf, y_buf, *scratch):
    pl.run_scoped(
        functools.partial(_compute, x_hbm, w_hbm, y_hbm, x_buf, y_buf, *scratch),
        pltpu.SemaphoreType.DMA((BANDS + 2,)),
        pltpu.SemaphoreType.DMA((READ_ITERS + 1,)),
    )
    pltpu.make_async_copy(y_buf.at[:, pl.ds(STEP, BAND_ROWS * C)], y_hbm, scratch[-1]).wait()


@jax.jit
def pallas_standalone__fft_conv__vision_kernel(x: jax.Array, w: jax.Array):
    assert x.shape == (1, H, W, C) and w.shape == (K, K, C, C)
    assert x.dtype == BF16 and w.dtype == BF16
    banded = (BANDS, BAND_ROWS * C, W)
    stage = pltpu.VMEM((BANDS, 6, C, 256), F32)
    ready = pltpu.VMEM((READY_ROUNDS * C // 2, 512), U32)
    y = pl.pallas_call(
        _kernel,
        in_specs=[pl.BlockSpec(memory_space=pl.ANY), pl.BlockSpec(memory_space=pl.ANY)],
        out_specs=pl.BlockSpec(memory_space=pl.ANY),
        out_shape=jax.ShapeDtypeStruct(banded, BF16),
        scratch_shapes=[
            pltpu.VMEM(banded, BF16),
            pltpu.VMEM((BANDS, STEP + BAND_ROWS * C, W), BF16),
            pltpu.VMEM((K, K, C, C), BF16),
            pltpu.VMEM((K, K, C, C), F32),
            pltpu.VMEM((6 * C // 2, 512), U32),
            stage, stage, ready, ready, stage, stage,
            pltpu.VMEM((BANDS, 2, C, 256), F32),
            pltpu.SemaphoreType.DMA(()),
        ],
        compiler_params=pltpu.CompilerParams(vmem_limit_bytes=64 * 2**20),
    )(jnp.transpose(x, (0, 1, 3, 2)).reshape(banded), w)
    return jnp.transpose(y.reshape(1, H, C, W), (0, 1, 3, 2))
```

```python
import functools

import jax
import jax.experimental.pallas as pl
import jax.experimental.pallas.tpu as pltpu
import jax.numpy as jnp
import numpy as np
from jax import lax

H, W, C, K = 224, 224, 96, 3
F32, BF16, U32 = jnp.float32, jnp.bfloat16, jnp.uint32

BANDS = 4
BAND_ROWS = H // BANDS
STEPS = BAND_ROWS // 4
SLABS = C // 16
STEP = 4 * C

A = (5.0**0.5 - 1.0) / 2.0
B = A + 1.0


def _filter_coefficients(p):
    norm = np.prod([p - q for q in (0.0, A, -A, B, -B) if q != p])
    return [float(p ** (k + 1) / norm) for k in range(K)]


DMA_ORDER = (0, 2, 1, 3)
READ_ITERS = 6
READ_ROWS = 7
EARLY_ROWS = BAND_ROWS - 2 - READ_ITERS * READ_ROWS
PIECE = 64
OLD_PIECES = 4
assert EARLY_ROWS == 12
assert OLD_PIECES * PIECE * (STEPS - 2 - READ_ITERS) == STEP * (READ_ITERS - 2)

READY_ROUNDS = 2
SLOT_AFTER = (0, 2, 3, 5)
IN_BAND_ORDER = (1, 2, 3, 0)
IN_DELAY, OUT_DELAY, READY_DELAY = 6, 4, 8


def _h_forward(d):
    s = d[2] * (A * A)
    p = d[4] - d[2] * (B * B)
    r = d[4] - s
    e = (d[3] - d[1]) * A
    q = e - d[1]
    u = e + d[3]
    return [d[0] + (p - s), p + q, p - q, r + u, r - u, (d[1] + d[5]) - d[3] * 3.0]


def _h_inverse(m):
    s1, d1 = m[1] + m[2], m[1] - m[2]
    s2, d2 = m[3] + m[4], m[3] - m[4]
    e = (s1 + s2) * A
    return [e + s1 + m[0], d1 + d2, e + s2, d1 * (A * A) + d2 * (B * B) + m[5]]


def _w_forward(t):
    d1, d2 = t[:, :128], t[:, 128:]
    return [pltpu.roll(d2, 2, 1) - d2, d1 + d2, d2 - d1, d1 - pltpu.roll(d1, 126, 1)]


def _w_inverse(p):
    return jnp.concatenate([p[0] + p[1] + p[2], p[1] - p[2] - p[3]], axis=1)


def _ds(start, size):
    return pl.ds(start if isinstance(start, int) else pl.multiple_of(start, 16), size)


def _slab(s):
    return pl.ds(16 * s, 16)


def _prepare_filter(w_buf, taps, u_buf):
    for a in range(K):
        for b in range(K):
            taps[a, b] = w_buf[K - 1 - a, K - 1 - b].astype(F32).T

    def body(s, _):
        rows = []
        for a in range(K):
            g0, g1, g2 = (taps[a, b, _ds(16 * s, 16), :] for b in range(K))
            even, odd = (g0 + g2) * 0.5, g1 * 0.5
            rows.append([g0, even + odd, even - odd, g2])
        for wc in range(4):
            g0, g1, g2 = (rows[a][wc] for a in range(K))
            parts = [g0]
            for p in (A, B):
                c0, c1, c2 = _filter_coefficients(p)
                even, odd = g0 * c0 + g2 * c2, g1 * c1
                parts += [even + odd, even - odd]
            parts.append(g2)
            for hc, u in enumerate(parts):
                u_buf[hc, wc, pl.ds(pl.multiple_of(8 * s, 8), 8), :] = pltpu.bitcast(u.astype(BF16), U32)

    lax.fori_loop(0, SLABS, body, None)


def _compute(
    x_hbm, w_hbm, y_hbm,
    x_buf, y_buf, w_buf, taps, u_buf, t_even, t_odd, v_even, v_odd, m_even, m_odd, carry,
    write_sem, early_sems, read_sems,
):
    all_bands = slice(None)

    def read(band, start, size, sem):
        where = (band, pl.ds(start, size))
        return pltpu.make_async_copy(x_hbm.at[where], x_buf.at[where], sem)

    def write(band, start, size):
        src, dst = y_buf.at[band, pl.ds(STEP + start, size)], y_hbm.at[band, pl.ds(start, size)]
        pltpu.make_async_copy(src, dst, write_sem).start()

    def first_rows(k):
        sem = early_sems.at[k]
        return read((k + BANDS - 1) % BANDS, (BAND_ROWS - 2) * C, 2 * C, sem), read(k, 0, STEP, sem)

    w_copy = pltpu.make_async_copy(w_hbm, w_buf, early_sems.at[BANDS + 1])
    w_copy.start()
    for k in range(BANDS):
        for copy in first_rows(k):
            copy.start()
    for k in range(BANDS):
        read(k, STEP, STEP, early_sems.at[BANDS]).start()
    for k in range(BANDS):
        read(k, 2 * STEP, STEP, read_sems.at[0]).start()

    def clear(k, _):
        m_odd[k] = jnp.zeros(m_odd.shape[1:], F32)

    lax.fori_loop(0, BANDS, clear, None)
    w_copy.wait()
    _prepare_filter(w_buf, taps, u_buf)

    def lane_masks(rows):
        lane = lax.broadcasted_iota(jnp.int32, (rows, 128), 1)
        return (lane & 1) == 0, (lane & 1) == 1, (lane >= 96) & (lane < 126), lane >= 126

    even, odd, middle, top = lane_masks(8)
    own_from_left, other_from_left = middle | (even ^ top), middle | (odd ^ top)
    even, _, _, top = lane_masks(16)
    left_is_first, right_is_second = even ^ top, even

    def load_right(ref, band, line):
        r = pltpu.bitcast(ref[band, pl.ds(line, 16), pl.ds(128, W - 128)], U32)
        return jnp.concatenate([r, r[:, 64:]], axis=1)

    def load_pixels(ref, band, line, right):
        left = pltpu.bitcast(ref[band, pl.ds(line, 16), pl.ds(0, 128)], U32)
        before = pltpu.roll(jnp.where(other_from_left, left, right), 1, 1)
        own = jnp.where(own_from_left, left, right)
        return jnp.concatenate([pltpu.bitcast(v, BF16).astype(F32) for v in (before, own)], axis=1)

    def store_pixels(ref, band, line, y):
        first, second = y[:, :128], pltpu.roll(y[:, 128:], 1, 1)
        left = jnp.where(left_is_first, first, second)
        right = jnp.where(right_is_second, second, first)[:, : W - 128]
        ref[band, pl.ds(line, 16), :] = jnp.concatenate([left, right], axis=1).astype(BF16)

    def keep(t_buf, v_buf, band, s, parts):
        for hc, t in enumerate(parts):
            if band == 0 and hc < READY_ROUNDS:
                v_buf[hc, _slab(s), :] = jnp.concatenate(_w_forward(t), axis=1).astype(BF16)
            else:
                t_buf[band, hc, _slab(s), :] = t

    def iteration(i, parity, reading=False):
        closing = isinstance(i, int)
        last = closing and i == STEPS
        t_new, t_old = (t_even, t_odd)[:: 1 - 2 * parity]
        v_new, v_old = (v_even, v_odd)[:: 1 - 2 * parity]
        m_old, m_new = (m_even, m_odd)[:: 1 - 2 * parity]
        units = 4 * SLABS * BANDS

        agenda = {}

        def plan(slot, fn, *args):
            agenda.setdefault(slot, []).append(functools.partial(fn, *args))

        def plan_forward():
            x_step = x_buf.at[:, _ds(STEP * i, STEP)]
            rights, rows = [], []

            def unit(j, band, s, r):
                if r == 0:
                    rows[:] = [carry[band, 0, _slab(s), :], carry[band, 1, _slab(s), :]]
                rows.append(load_pixels(x_step, band, r * C + 16 * s, rights.pop(0)))
                if r == 3:
                    carry[band, 0, _slab(s), :] = rows[4]
                    carry[band, 1, _slab(s), :] = rows[5]
                    args = (t_new, v_new, band, s, _h_forward(rows))
                    if band == 0:
                        plan(j + IN_DELAY + READY_DELAY, keep, *args)
                    else:
                        keep(*args)

            for j in range(units):
                band, s, r = IN_BAND_ORDER[j // (4 * SLABS)], j // 4 % SLABS, j % 4
                plan(j, lambda *a: rights.append(load_right(*a)), x_step, band, r * C + 16 * s)
                plan(j + IN_DELAY, unit, j, band, s, r)

        def plan_inverse(m_buf, step, slot, band_major):
            y_step = y_buf.at[:, _ds(STEP * (step + 1), STEP)]
            rows = []

            def unit(j):
                r = j % 4
                band, s = (j // (4 * SLABS), j // 4 % SLABS) if band_major else (j // 4 % BANDS, j // (4 * BANDS))
                if r == 0:
                    rows[:] = _h_inverse([m_buf[band, hc, _slab(s), :] for hc in range(6)])
                store_pixels(y_step, band, r * C + 16 * s, rows[r])
                if closing and (j + 1) % (units // 2) == 0:
                    for line in range(STEP * step, STEP * (step + 1), C):
                        if band_major:
                            write(band - 1, line, C)
                            write(band, line, C)
                        else:
                            for k in DMA_ORDER:
                                write(k, line + 16 * (s + 1) - C // 2, C // 2)

            for j in range(units):
                plan(slot(j), unit, j)

        if last:
            plan_inverse(m_old, i - 2, lambda j: j // 2, False)
            plan_inverse(m_new, i - 1, lambda j: max(48 + j // 2, 24 * (j // 24) + 36 + j % 24 // 2), True)
        else:
            plan_forward()
            plan_inverse(m_old, i - 2, lambda j: j + OUT_DELAY, not closing)

        def start_piece(src, dst, n, size, sem, priority):
            where = (DMA_ORDER[n % BANDS], pl.ds(n // BANDS * size, size))
            pltpu.make_async_copy(src.at[where], dst.at[where], sem).start(priority=priority)

        if reading:
            span = _ds((EARLY_ROWS + (i - 1) * READ_ROWS) * C, READ_ROWS * C)
            count = BANDS * READ_ROWS
            for n in range(count):
                args = (x_hbm.at[:, span], x_buf.at[:, span], n, C, read_sems.at[i], n % 2)
                plan(n * 100 // count, start_piece, *args)
        elif not closing:
            spans = [((i - READ_ITERS - 1) * OLD_PIECES * PIECE, OLD_PIECES * PIECE), ((i - 3) * STEP, STEP)]
            pieces = sorted(
                ((n + 0.5) * PIECE / size, which, n)
                for which, (_, size) in enumerate(spans)
                for n in range(size // PIECE)
            )
            count = BANDS * len(pieces)
            for n in range(count):
                _, which, piece = pieces[n // BANDS]
                start, size = spans[which]
                src, dst = y_buf.at[:, _ds(STEP + start, size)], y_hbm.at[:, _ds(start, size)]
                plan(12 + n * 68 // count, start_piece, src, dst, BANDS * piece + n % BANDS, PIECE, write_sem, 0)
        elif not last:
            count = BANDS * STEP // PIECE
            for n in range(count):
                plan(n * 32 // count, write, DMA_ORDER[n % BANDS], (i - 3) * STEP + n // BANDS * PIECE, PIECE)

        slot = 0

        def emit():
            nonlocal slot
            for fn in agenda.pop(slot, []):
                fn()
            slot += 1

        for band in range(BANDS):
            for hc in range(6):
                if band == 0 and hc < READY_ROUNDS:
                    v = [v_old[hc, :, pl.ds(128 * wc, 128)] for wc in range(4)]
                    for _ in SLOT_AFTER:
                        emit()
                else:
                    slabs = []
                    for n in range(SLABS):
                        slabs.insert(0, _w_forward(t_old[band, hc, _slab(SLABS - 1 - n), :]))
                        if n in SLOT_AFTER:
                            emit()
                    v = [jnp.concatenate(part, axis=0).astype(BF16) for part in zip(*slabs)]
                m_new[band, hc] = _w_inverse([
                    jnp.dot(pltpu.bitcast(u_buf[hc, wc], BF16), v[wc], preferred_element_type=F32)
                    for wc in range(4)
                ])
        while agenda:
            emit()

    def first_step(k, _):
        for copy in first_rows(k):
            copy.wait()
        above = (k + BANDS - 1) % BANDS
        lines = [(above, (BAND_ROWS - 2 + r) * C) for r in range(2)] + [(k, r * C) for r in range(4)]
        rights = [[load_right(x_buf, band, line + 16 * s) for band, line in lines] for s in range(SLABS)]
        for s in range(SLABS):
            rows = [load_pixels(x_buf, band, line + 16 * s, r) for (band, line), r in zip(lines, rights[s])]
            carry[k, 0, _slab(s), :] = rows[4]
            carry[k, 1, _slab(s), :] = rows[5]
            for hc, t in enumerate(_h_forward(rows)):
                t_even[k, hc, _slab(s), :] = t

    lax.fori_loop(0, BANDS, first_step, None)
    for s in range(SLABS):
        keep(t_even, v_even, 0, s, [t_even[0, hc, _slab(s), :] for hc in range(READY_ROUNDS)])
    read(all_bands, STEP, STEP, early_sems.at[BANDS]).wait()

    edges = [8] + [EARLY_ROWS + b * READ_ROWS for b in range(READ_ITERS + 1)]
    assert all(b < edges[b] // 4 < STEPS - 1 for b in range(READ_ITERS + 1))

    def run(begin, end, reading):
        def body(i, _):
            for b, (lo, hi) in enumerate(zip(edges, edges[1:])):
                if begin <= lo // 4 < end:
                    pl.when(i == lo // 4)(read(all_bands, lo * C, (hi - lo) * C, read_sems.at[b]).wait)
            lax.cond((i & 1) == 0, lambda: iteration(i, 0, reading), lambda: iteration(i, 1, reading))

        lax.fori_loop(begin, end, body, None)

    run(1, READ_ITERS + 1, True)
    run(READ_ITERS + 1, STEPS - 1, False)
    closing = [functools.partial(iteration, i, i % 2) for i in (STEPS - 1, STEPS)]
    lax.fori_loop(0, 2, lambda n, _: lax.switch(n, closing), None)


def _kernel(x_hbm, w_hbm, y_hbm, x_buf, y_buf, *scratch):
    pl.run_scoped(
        functools.partial(_compute, x_hbm, w_hbm, y_hbm, x_buf, y_buf, *scratch),
        pltpu.SemaphoreType.DMA((BANDS + 2,)),
        pltpu.SemaphoreType.DMA((READ_ITERS + 1,)),
    )
    pltpu.make_async_copy(y_buf.at[:, pl.ds(STEP, BAND_ROWS * C)], y_hbm, scratch[-1]).wait()


@jax.jit
def pallas_standalone__fft_conv__vision_kernel(x: jax.Array, w: jax.Array):
    assert x.shape == (1, H, W, C) and w.shape == (K, K, C, C)
    assert x.dtype == BF16 and w.dtype == BF16
    banded = (BANDS, BAND_ROWS * C, W)
    stage = pltpu.VMEM((BANDS, 6, C, 256), F32)
    ready = pltpu.VMEM((READY_ROUNDS, C, 512), BF16)
    y = pl.pallas_call(
        _kernel,
        in_specs=[pl.BlockSpec(memory_space=pl.ANY), pl.BlockSpec(memory_space=pl.ANY)],
        out_specs=pl.BlockSpec(memory_space=pl.ANY),
        out_shape=jax.ShapeDtypeStruct(banded, BF16),
        scratch_shapes=[
            pltpu.VMEM(banded, BF16),
            pltpu.VMEM((BANDS, STEP + BAND_ROWS * C, W), BF16),
            pltpu.VMEM((K, K, C, C), BF16),
            pltpu.VMEM((K, K, C, C), F32),
            pltpu.VMEM((6, 4, C // 2, C), U32),
            stage, stage, ready, ready, stage, stage,
            pltpu.VMEM((BANDS, 2, C, 256), F32),
            pltpu.SemaphoreType.DMA(()),
        ],
        compiler_params=pltpu.CompilerParams(vmem_limit_bytes=64 * 2**20),
    )(jnp.transpose(x, (0, 1, 3, 2)).reshape(banded), w)
    return jnp.transpose(y.reshape(1, H, C, W), (0, 1, 3, 2))
```

```python
import functools

import jax
import jax.experimental.pallas as pl
import jax.experimental.pallas.tpu as pltpu
import jax.numpy as jnp
import numpy as np
from jax import lax

H, W, C, K = 224, 224, 96, 3
F32, BF16, U32 = jnp.float32, jnp.bfloat16, jnp.uint32

BANDS = 4
BAND_ROWS = H // BANDS
STEPS = BAND_ROWS // 4
SLABS = C // 16
STEP = 4 * C

A = (5.0**0.5 - 1.0) / 2.0
B = A + 1.0


def _filter_coefficients(p):
    norm = np.prod([p - q for q in (0.0, A, -A, B, -B) if q != p])
    return [float(p ** (k + 1) / norm) for k in range(K)]


DMA_ORDER = (0, 2, 1, 3)
READ_ITERS = 6
READ_ROWS = 7
EARLY_ROWS = BAND_ROWS - 2 - READ_ITERS * READ_ROWS
PIECE = 64
OLD_PIECES = 4
assert EARLY_ROWS == 12
assert OLD_PIECES * PIECE * (STEPS - 2 - READ_ITERS) == STEP * (READ_ITERS - 2)

READY_ROUNDS = 2
SLOT_AFTER = (0, 1, 3, 4)
IN_BAND_ORDER = (1, 2, 3, 0)
WRITE_BEGIN, WRITE_SLOTS = 28, 62
IN_DELAY, OUT_DELAY, READY_DELAY = 6, 12, 8


def _h_forward(d):
    s = d[2] * (A * A)
    p = d[4] - d[2] * (B * B)
    r = d[4] - s
    e = (d[3] - d[1]) * A
    q = e - d[1]
    u = e + d[3]
    return [d[0] + (p - s), p + q, p - q, r + u, r - u, (d[1] + d[5]) - d[3] * 3.0]


def _h_inverse(m):
    s1, d1 = m[1] + m[2], m[1] - m[2]
    s2, d2 = m[3] + m[4], m[3] - m[4]
    e = (s1 + s2) * A
    return [e + s1 + m[0], d1 + d2, e + s2, d1 * (A * A) + d2 * (B * B) + m[5]]


def _w_forward(t):
    d1, d2 = t[:, :128], t[:, 128:]
    return [pltpu.roll(d2, 2, 1) - d2, d1 + d2, d2 - d1, d1 - pltpu.roll(d1, 126, 1)]


def _w_inverse(p):
    return jnp.concatenate([p[0] + p[1] + p[2], p[1] - p[2] - p[3]], axis=1)


def _ds(start, size):
    return pl.ds(start if isinstance(start, int) else pl.multiple_of(start, 16), size)


def _slab(s):
    return pl.ds(16 * s, 16)


def _prepare_filter(w_buf, taps, u_buf):
    for a in range(K):
        for b in range(K):
            taps[a, b] = w_buf[K - 1 - a, K - 1 - b].astype(F32).T

    def body(s, _):
        rows = []
        for a in range(K):
            g0, g1, g2 = (taps[a, b, _ds(16 * s, 16), :] for b in range(K))
            even, odd = (g0 + g2) * 0.5, g1 * 0.5
            rows.append([g0, even + odd, even - odd, g2])
        for wc in range(4):
            g0, g1, g2 = (rows[a][wc] for a in range(K))
            parts = [g0]
            for p in (A, B):
                c0, c1, c2 = _filter_coefficients(p)
                even, odd = g0 * c0 + g2 * c2, g1 * c1
                parts += [even + odd, even - odd]
            parts.append(g2)
            for hc, u in enumerate(parts):
                u_buf[hc, wc, pl.ds(pl.multiple_of(8 * s, 8), 8), :] = pltpu.bitcast(u.astype(BF16), U32)

    lax.fori_loop(0, SLABS, body, None)


def _compute(
    x_hbm, w_hbm, y_hbm,
    x_buf, y_buf, w_buf, taps, u_buf, t_even, t_odd, v_even, v_odd, m_even, m_odd, carry,
    write_sem, early_sems, read_sems,
):
    all_bands = slice(None)

    def read(band, start, size, sem):
        where = (band, pl.ds(start, size))
        return pltpu.make_async_copy(x_hbm.at[where], x_buf.at[where], sem)

    def write(band, start, size):
        src, dst = y_buf.at[band, pl.ds(STEP + start, size)], y_hbm.at[band, pl.ds(start, size)]
        pltpu.make_async_copy(src, dst, write_sem).start()

    def first_rows(k):
        sem = early_sems.at[k]
        return read((k + BANDS - 1) % BANDS, (BAND_ROWS - 2) * C, 2 * C, sem), read(k, 0, STEP, sem)

    w_copy = pltpu.make_async_copy(w_hbm, w_buf, early_sems.at[BANDS + 1])
    w_copy.start()
    for k in range(BANDS):
        for copy in first_rows(k):
            copy.start()
    for k in range(BANDS):
        read(k, STEP, STEP, early_sems.at[BANDS]).start()
    for k in range(BANDS):
        read(k, 2 * STEP, STEP, read_sems.at[0]).start()

    def clear(k, _):
        m_odd[k] = jnp.zeros(m_odd.shape[1:], F32)

    lax.fori_loop(0, BANDS, clear, None)
    w_copy.wait()
    _prepare_filter(w_buf, taps, u_buf)

    def lane_masks(rows):
        lane = lax.broadcasted_iota(jnp.int32, (rows, 128), 1)
        return (lane & 1) == 0, (lane & 1) == 1, (lane >= 96) & (lane < 126), lane >= 126

    even, odd, middle, top = lane_masks(8)
    own_from_left, other_from_left = middle | (even ^ top), middle | (odd ^ top)
    even, _, _, top = lane_masks(16)
    left_is_first, right_is_second = even ^ top, even

    def load_right(ref, band, line):
        r = pltpu.bitcast(ref[band, pl.ds(line, 16), pl.ds(128, W - 128)], U32)
        return jnp.concatenate([r, r[:, 64:]], axis=1)

    def load_pixels(ref, band, line, right):
        left = pltpu.bitcast(ref[band, pl.ds(line, 16), pl.ds(0, 128)], U32)
        before = pltpu.roll(jnp.where(other_from_left, left, right), 1, 1)
        own = jnp.where(own_from_left, left, right)
        return jnp.concatenate([pltpu.bitcast(v, BF16).astype(F32) for v in (before, own)], axis=1)

    def store_pixels(ref, band, line, y):
        first, second = y[:, :128], pltpu.roll(y[:, 128:], 1, 1)
        left = jnp.where(left_is_first, first, second)
        right = jnp.where(right_is_second, second, first)[:, : W - 128]
        ref[band, pl.ds(line, 16), :] = jnp.concatenate([left, right], axis=1).astype(BF16)

    def keep(t_buf, v_buf, band, s, parts):
        for hc, t in enumerate(parts):
            if band == 0 and hc < READY_ROUNDS:
                v_buf[hc, _slab(s), :] = jnp.concatenate(_w_forward(t), axis=1).astype(BF16)
            else:
                t_buf[band, hc, _slab(s), :] = t

    def iteration(i, parity, reading=False):
        closing = isinstance(i, int)
        last = closing and i == STEPS
        t_new, t_old = (t_even, t_odd)[:: 1 - 2 * parity]
        v_new, v_old = (v_even, v_odd)[:: 1 - 2 * parity]
        m_old, m_new = (m_even, m_odd)[:: 1 - 2 * parity]
        units = 4 * SLABS * BANDS

        agenda = {}

        def plan(slot, fn, *args):
            agenda.setdefault(slot, []).append(functools.partial(fn, *args))

        def plan_forward():
            x_step = x_buf.at[:, _ds(STEP * i, STEP)]
            rights, rows = [], []

            def unit(j, band, s, r):
                if r == 0:
                    rows[:] = [carry[band, 0, _slab(s), :], carry[band, 1, _slab(s), :]]
                rows.append(load_pixels(x_step, band, r * C + 16 * s, rights.pop(0)))
                if r == 3:
                    carry[band, 0, _slab(s), :] = rows[4]
                    carry[band, 1, _slab(s), :] = rows[5]
                    args = (t_new, v_new, band, s, _h_forward(rows))
                    if band == 0:
                        plan(j + IN_DELAY + READY_DELAY, keep, *args)
                    else:
                        keep(*args)

            for j in range(units):
                band, s, r = IN_BAND_ORDER[j // (4 * SLABS)], j // 4 % SLABS, j % 4
                plan(j, lambda *a: rights.append(load_right(*a)), x_step, band, r * C + 16 * s)
                plan(j + IN_DELAY, unit, j, band, s, r)

        def plan_inverse(m_buf, step, slot, band_major):
            y_step = y_buf.at[:, _ds(STEP * (step + 1), STEP)]
            rows = []

            def unit(j):
                r = j % 4
                band, s = (j // (4 * SLABS), j // 4 % SLABS) if band_major else (j // 4 % BANDS, j // (4 * BANDS))
                if r == 0:
                    rows[:] = _h_inverse([m_buf[band, hc, _slab(s), :] for hc in range(6)])
                store_pixels(y_step, band, r * C + 16 * s, rows[r])
                if closing and (j + 1) % (units // 2) == 0:
                    for line in range(STEP * step, STEP * (step + 1), C):
                        if band_major:
                            write(band - 1, line, C)
                            write(band, line, C)
                        else:
                            for k in DMA_ORDER:
                                write(k, line + 16 * (s + 1) - C // 2, C // 2)

            for j in range(units):
                plan(slot(j), unit, j)

        if last:
            plan_inverse(m_old, i - 2, lambda j: j // 2, False)
            plan_inverse(m_new, i - 1, lambda j: max(48 + j // 2, 24 * (j // 24) + 36 + j % 24 // 2), True)
        else:
            plan_forward()
            plan_inverse(m_old, i - 2, lambda j: j + OUT_DELAY, not closing)

        def start_piece(src, dst, n, size, sem, priority):
            where = (DMA_ORDER[n % BANDS], pl.ds(n // BANDS * size, size))
            pltpu.make_async_copy(src.at[where], dst.at[where], sem).start(priority=priority)

        if reading:
            span = _ds((EARLY_ROWS + (i - 1) * READ_ROWS) * C, READ_ROWS * C)
            count = BANDS * READ_ROWS
            for n in range(count):
                args = (x_hbm.at[:, span], x_buf.at[:, span], n, C, read_sems.at[i], n % 2)
                plan(n * 100 // count, start_piece, *args)
        elif not closing:
            spans = [((i - READ_ITERS - 1) * OLD_PIECES * PIECE, OLD_PIECES * PIECE), ((i - 3) * STEP, STEP)]
            pieces = sorted(
                ((n + 0.5) * PIECE / size, which, n)
                for which, (_, size) in enumerate(spans)
                for n in range(size // PIECE)
            )
            count = BANDS * len(pieces)
            for n in range(count):
                _, which, piece = pieces[n // BANDS]
                start, size = spans[which]
                src, dst = y_buf.at[:, _ds(STEP + start, size)], y_hbm.at[:, _ds(start, size)]
                args = (src, dst, BANDS * piece + n % BANDS, PIECE, write_sem, 0)
                plan(WRITE_BEGIN + n * WRITE_SLOTS // count, start_piece, *args)
        elif not last:
            count = BANDS * STEP // PIECE
            for n in range(count):
                plan(n * 32 // count, write, DMA_ORDER[n % BANDS], (i - 3) * STEP + n // BANDS * PIECE, PIECE)

        slot = 0

        def emit():
            nonlocal slot
            for fn in agenda.pop(slot, []):
                fn()
            slot += 1

        for band in range(BANDS):
            for hc in range(6):
                if band == 0 and hc < READY_ROUNDS:
                    v = [v_old[hc, :, pl.ds(128 * wc, 128)] for wc in range(4)]
                    for _ in SLOT_AFTER:
                        emit()
                else:
                    slabs = []
                    for n in range(SLABS):
                        slabs.insert(0, _w_forward(t_old[band, hc, _slab(SLABS - 1 - n), :]))
                        if n in SLOT_AFTER:
                            emit()
                    v = [jnp.concatenate(part, axis=0).astype(BF16) for part in zip(*slabs)]
                m_new[band, hc] = _w_inverse([
                    jnp.dot(pltpu.bitcast(u_buf[hc, wc], BF16), v[wc], preferred_element_type=F32)
                    for wc in range(4)
                ])
        while agenda:
            emit()

    def first_step(k, _):
        for copy in first_rows(k):
            copy.wait()
        above = (k + BANDS - 1) % BANDS
        lines = [(above, (BAND_ROWS - 2 + r) * C) for r in range(2)] + [(k, r * C) for r in range(4)]
        rights = [[load_right(x_buf, band, line + 16 * s) for band, line in lines] for s in range(SLABS)]
        for s in range(SLABS):
            rows = [load_pixels(x_buf, band, line + 16 * s, r) for (band, line), r in zip(lines, rights[s])]
            carry[k, 0, _slab(s), :] = rows[4]
            carry[k, 1, _slab(s), :] = rows[5]
            for hc, t in enumerate(_h_forward(rows)):
                t_even[k, hc, _slab(s), :] = t

    lax.fori_loop(0, BANDS, first_step, None)
    for s in range(SLABS):
        keep(t_even, v_even, 0, s, [t_even[0, hc, _slab(s), :] for hc in range(READY_ROUNDS)])
    read(all_bands, STEP, STEP, early_sems.at[BANDS]).wait()

    edges = [8] + [EARLY_ROWS + b * READ_ROWS for b in range(READ_ITERS + 1)]
    assert all(b < edges[b] // 4 < STEPS - 1 for b in range(READ_ITERS + 1))

    def run(begin, end, reading):
        def body(i, _):
            for b, (lo, hi) in enumerate(zip(edges, edges[1:])):
                if begin <= lo // 4 < end:
                    pl.when(i == lo // 4)(read(all_bands, lo * C, (hi - lo) * C, read_sems.at[b]).wait)
            lax.cond((i & 1) == 0, lambda: iteration(i, 0, reading), lambda: iteration(i, 1, reading))

        lax.fori_loop(begin, end, body, None)

    run(1, READ_ITERS + 1, True)
    run(READ_ITERS + 1, STEPS - 1, False)
    closing = [functools.partial(iteration, i, i % 2) for i in (STEPS - 1, STEPS)]
    lax.fori_loop(0, 2, lambda n, _: lax.switch(n, closing), None)


def _kernel(x_hbm, w_hbm, y_hbm, x_buf, y_buf, *scratch):
    pl.run_scoped(
        functools.partial(_compute, x_hbm, w_hbm, y_hbm, x_buf, y_buf, *scratch),
        pltpu.SemaphoreType.DMA((BANDS + 2,)),
        pltpu.SemaphoreType.DMA((READ_ITERS + 1,)),
    )
    pltpu.make_async_copy(y_buf.at[:, pl.ds(STEP, BAND_ROWS * C)], y_hbm, scratch[-1]).wait()


@jax.jit
def pallas_standalone__fft_conv__vision_kernel(x: jax.Array, w: jax.Array):
    assert x.shape == (1, H, W, C) and w.shape == (K, K, C, C)
    assert x.dtype == BF16 and w.dtype == BF16
    banded = (BANDS, BAND_ROWS * C, W)
    stage = pltpu.VMEM((BANDS, 6, C, 256), F32)
    ready = pltpu.VMEM((READY_ROUNDS, C, 512), BF16)
    y = pl.pallas_call(
        _kernel,
        in_specs=[pl.BlockSpec(memory_space=pl.ANY), pl.BlockSpec(memory_space=pl.ANY)],
        out_specs=pl.BlockSpec(memory_space=pl.ANY),
        out_shape=jax.ShapeDtypeStruct(banded, BF16),
        scratch_shapes=[
            pltpu.VMEM(banded, BF16),
            pltpu.VMEM((BANDS, STEP + BAND_ROWS * C, W), BF16),
            pltpu.VMEM((K, K, C, C), BF16),
            pltpu.VMEM((K, K, C, C), F32),
            pltpu.VMEM((6, 4, C // 2, C), U32),
            stage, stage, ready, ready, stage, stage,
            pltpu.VMEM((BANDS, 2, C, 256), F32),
            pltpu.SemaphoreType.DMA(()),
        ],
        compiler_params=pltpu.CompilerParams(vmem_limit_bytes=64 * 2**20),
    )(jnp.transpose(x, (0, 1, 3, 2)).reshape(banded), w)
    return jnp.transpose(y.reshape(1, H, C, W), (0, 1, 3, 2))
```
